```python
import jax
import jax.numpy as jnp

def _softmax(x, axis=-1):
    return jax.nn.softmax(x, axis=axis)
def _gelu(x):
    return jax.nn.gelu(x, approximate=True)
def _silu(x):
    return jax.nn.silu(x)
def _sigmoid(x):
    return jax.nn.sigmoid(x)
def _layernorm(x, axis=-1, eps=1e-5):
    m = jnp.mean(x, axis=axis, keepdims=True)
    v = jnp.var(x, axis=axis, keepdims=True)
    return (x - m) / jnp.sqrt(v + eps)
def _scatter_add(tgt, idx, src, axis=0):
    return tgt.at[idx].add(src)
def _segment_sum(src, seg, n):
    return jax.ops.segment_sum(src, seg, n)
class _Rng:
    def __init__(self, key):
        self._k = key
    def _next(self):
        self._k, sub = jax.random.split(self._k)
        return sub
    def normal(self, shape):
        return jax.random.normal(self._next(), shape, dtype=jnp.bfloat16)
    def randint(self, lo, hi, shape):
        return jax.random.randint(self._next(), shape, lo, hi, dtype=jnp.int32)
    def uniform(self, shape, lo=0.0, hi=1.0):
        return jax.random.uniform(self._next(), shape, jnp.bfloat16, lo, hi)
    def permutation(self, n):
        return jax.random.permutation(self._next(), n)


kernel_name = 'standalone__standard_2d_1d_3d_conv__vision'

def setup_inputs():
    _rng = _Rng(jax.random.key(int.from_bytes(__import__("os").urandom(4), "little")))
    _w = (lambda a: (lambda t: t.astype(jnp.bfloat16) if jnp.issubdtype(t.dtype, jnp.floating) else t)(jnp.asarray(a)))
    H = W = 384
    C = 384
    K = 1
    return {
        "x": _w((lambda *s: _rng.normal(s) * 0.05)(1, H, W, C)),
        "w": _w((lambda *s: _rng.normal(s) * 0.05)(K, K, C, C)),
        "b": _w((lambda *s: _rng.normal(s) * 0.05)(C)),
    }

def reference(x, w, b):
    B, H, W, Cin = x.shape
    K = w.shape[0]
    pl = (K - 1) // 2
    pr = K // 2
    xp = jnp.pad(x, ((0, 0), (pl, pr), (pl, pr), (0, 0)))
    out = sum(
        jnp.einsum('bhwc,cd->bhwd', xp[:, i:i+H, j:j+W, :], w[i, j])
        for i in range(K) for j in range(K)
    )
    return out + b[None, None, None, :]
```

```python
import jax
import jax.numpy as jnp
import jax.experimental.pallas as pl
import jax.experimental.pallas.tpu as pltpu
from jax import lax

_G = 6
_WR = 48
_RR = 384
_CR = 384
_PRE_R = 4
_PRE_W = 2


@jax.jit
def pallas_standalone__standard_2d_1d_3d_conv__vision_kernel(
    x: jax.Array,
    w: jax.Array,
    b: jax.Array,
):
    B, H, W, C = x.shape
    assert w.shape == (1, 1, C, C)
    M = B * H * W
    R = M // _G
    n = R // _RR
    assert R * _G == M and n * _RR == R
    half = n // 2
    writes_per_chunk = _RR // _WR

    def kernel_function(x_hbm, w_hbm, b_hbm, o_hbm, buf, w_v, b_v, rsem, wsem, csem):
        def read(i):
            rows = pl.ds(pl.multiple_of(i * _RR, _RR), _RR)
            return pltpu.make_async_copy(x_hbm.at[:, rows], buf.at[:, rows], rsem.at[i])

        def start_writes(i):
            for k in range(writes_per_chunk):
                rows = pl.ds(pl.multiple_of(i * _RR + k * _WR, _WR), _WR)
                pltpu.make_async_copy(buf.at[:, rows], o_hbm.at[:, rows], wsem).start()

        def compute(i):
            def tile(t, _):
                rows = pl.ds(pl.multiple_of(i * _RR + t * _CR, _CR), _CR)
                xv = buf[:, rows, :].reshape(_G * _CR, C)
                acc = jnp.dot(xv, w_v[...], preferred_element_type=jnp.float32)
                acc = acc + b_v[...].astype(jnp.float32).reshape(1, C)
                buf[:, rows, :] = acc.astype(buf.dtype).reshape(_G, _CR, C)

            lax.fori_loop(0, _RR // _CR, tile, None)

        copy_w = pltpu.make_async_copy(w_hbm, w_v, csem.at[0])
        copy_b = pltpu.make_async_copy(b_hbm, b_v, csem.at[1])
        read(0).start()
        copy_w.start()
        copy_b.start()
        for i in range(1, _PRE_R):
            read(i).start()
        copy_w.wait()
        copy_b.wait()

        def phase1(i, _):
            for q in range(2):
                j = _PRE_R + 2 * i + q
                pl.when(j < n)(lambda: read(j).start())
            read(i).wait()
            compute(i)

        lax.fori_loop(0, half, phase1, None)
        lax.fori_loop(half, n, lambda i, _: read(i).wait(), None)

        for c in range(_PRE_W):
            start_writes(c)

        def phase2(i, issued):
            compute(i)
            target = jnp.minimum(i + 1, _PRE_W + 2 * (i - half + 1))
            lax.fori_loop(issued, target, lambda c, _: start_writes(c), None)
            return target

        lax.fori_loop(half, n, phase2, jnp.int32(_PRE_W))
        pltpu.make_async_copy(buf, o_hbm, wsem).wait()

    any_spec = pl.BlockSpec(memory_space=pl.ANY)
    out = pl.pallas_call(
        kernel_function,
        in_specs=[any_spec, any_spec, any_spec],
        out_specs=any_spec,
        out_shape=jax.ShapeDtypeStruct((_G, R, C), x.dtype),
        scratch_shapes=[
            pltpu.VMEM((_G, R, C), x.dtype),
            pltpu.VMEM((C, C), w.dtype),
            pltpu.VMEM((C,), b.dtype),
            pltpu.SemaphoreType.DMA((n,)),
            pltpu.SemaphoreType.DMA(()),
            pltpu.SemaphoreType.DMA((2,)),
        ],
        compiler_params=pltpu.CompilerParams(vmem_limit_bytes=120 * 1024 * 1024),
    )(x.reshape(_G, R, C), w.reshape(C, C), b)
    return out.reshape(B, H, W, C)
```

```python
import jax
import jax.numpy as jnp
import jax.experimental.pallas as pl
import jax.experimental.pallas.tpu as pltpu
from jax import lax

_G = 6
_P = 4096
_BLOCK = 128
_DMA = 32
_SMALL = 16
_STEPS = 96
_BULK = 7
_AHEAD = 2
_SWITCH = 3
_PRE_WRITE = 2


@jax.jit
def pallas_standalone__standard_2d_1d_3d_conv__vision_kernel(
    x: jax.Array,
    w: jax.Array,
    b: jax.Array,
):
    B, H, W, C = x.shape
    assert w.shape == (1, 1, C, C) and C % 128 == 0
    sections = B * H * W // (_G * _P)
    assert sections * _G * _P == B * H * W
    blocks_per_section = _P // _BLOCK
    blocks = sections * blocks_per_section
    dmas_per_section = _P // _DMA
    dmas_per_block = _BLOCK // _DMA
    small_start = _STEPS * _BULK * _DMA - (sections - 1) * _P
    small_per_group = (_P - small_start) // (_STEPS * _SMALL)
    assert 0 <= small_start and small_start + small_per_group * _STEPS * _SMALL == _P
    lane_tiles = C // 128

    def kernel_function(x_hbm, w_hbm, b_hbm, o_hbm, buf, w_v, b_v,
                        bulk_sem, last_sem, small_sem, write_sem, param_sem):
        def dma_slice(m):
            if isinstance(m, int):
                return (m // dmas_per_section, slice(None),
                        pl.ds(m % dmas_per_section * _DMA, _DMA))
            start = pl.multiple_of(lax.rem(m, dmas_per_section) * _DMA, _DMA)
            return lax.div(m, dmas_per_section), slice(None), pl.ds(start, _DMA)

        def bulk_read(m, sem):
            ix = dma_slice(m)
            return pltpu.make_async_copy(x_hbm.at[ix], buf.at[ix], sem)

        def small_read(step, g, q):
            start = small_start + (step * small_per_group + q) * _SMALL
            if not isinstance(start, int):
                start = pl.multiple_of(start, _SMALL)
            ix = (sections - 1, g, pl.ds(start, _SMALL))
            pltpu.make_async_copy(x_hbm.at[ix], buf.at[ix], small_sem).start(priority=0)

        def write_block(k):
            for q in range(dmas_per_block):
                ix = dma_slice(k * dmas_per_block + q)
                pltpu.make_async_copy(buf.at[ix], o_hbm.at[ix], write_sem).start()

        def block_rows(k):
            start = pl.multiple_of(lax.rem(k, blocks_per_section) * _BLOCK, _BLOCK)
            return lax.div(k, blocks_per_section), pl.ds(start, _BLOCK)

        def conv(xv):
            acc = jnp.dot(xv, w_v[...], preferred_element_type=jnp.float32)
            acc = acc + b_v[...].astype(jnp.float32).reshape(1, C)
            return acc.astype(buf.dtype)

        def compute(k):
            s, rows = block_rows(k)
            xv = buf[s, :, rows, :].reshape(_G * _BLOCK, C)
            buf[s, :, rows, :] = conv(xv).reshape(_G, _BLOCK, C)

        def compute_and_read(k, step):
            s, rows = block_rows(k)
            xv = buf[s, 0, rows, :]
            for g in range(_G):
                nxt = buf[s, g + 1, rows, :] if g + 1 < _G else None
                y = conv(xv)
                q = 0
                for c in range(lane_tiles):
                    lanes = slice(c * 128, (c + 1) * 128)
                    buf[s, g, rows, lanes] = y[:, lanes]
                    while (q + 1) * lane_tiles <= (c + 1) * small_per_group:
                        small_read(step, g, q)
                        q += 1
                xv = nxt

        copy_w = pltpu.make_async_copy(w_hbm, w_v, param_sem.at[0])
        copy_b = pltpu.make_async_copy(b_hbm, b_v, param_sem.at[1])
        for i in range(_AHEAD):
            for q in range(_BULK):
                bulk_read(i * _BULK + q, bulk_sem.at[i]).start(priority=1)
            if i == 0:
                copy_w.start()
                copy_b.start()
        for g in range(_G):
            for q in range(small_per_group):
                pl.delay(110)
                small_read(0, g, q)
        copy_w.wait()
        copy_b.wait()

        def read_step(i, _):
            for q in range(_BULK):
                bulk_read(q, bulk_sem.at[lax.rem(i, _AHEAD + 1)]).wait()
            j = i + _AHEAD

            @pl.when(j < _STEPS - 1)
            def _():
                for q in range(_BULK):
                    sem = bulk_sem.at[lax.rem(j, _AHEAD + 1)]
                    bulk_read(j * _BULK + q, sem).start(priority=1)

            @pl.when(j == _STEPS - 1)
            def _():
                for q in range(_BULK):
                    bulk_read((_STEPS - 1) * _BULK + q, last_sem.at[q]).start(priority=1)

            compute_and_read(i, i + 1)

        lax.fori_loop(0, _STEPS - 1, read_step, None)

        for q in range(_SWITCH):
            bulk_read(q, last_sem.at[q]).wait()
        for k in range(_PRE_WRITE):
            write_block(k)
        for q in range(_SWITCH, _BULK):
            bulk_read(q, last_sem.at[q]).wait()
        small = (sections - 1, slice(None), pl.ds(small_start, _P - small_start))
        pltpu.make_async_copy(x_hbm.at[small], buf.at[small], small_sem).wait()

        first = _STEPS - 1
        assert _PRE_WRITE + 2 * (blocks - first) >= blocks

        def write_step(k, written):
            compute(k)
            target = jnp.minimum(k + 1, _PRE_WRITE + 2 * (k + 1 - first))
            lax.fori_loop(written, target, lambda c, _: write_block(c), None)
            return target

        lax.fori_loop(first, blocks, write_step, jnp.int32(_PRE_WRITE))
        pltpu.make_async_copy(buf, o_hbm, write_sem).wait()

    any_spec = pl.BlockSpec(memory_space=pl.ANY)
    out = pl.pallas_call(
        kernel_function,
        in_specs=[any_spec, any_spec, any_spec],
        out_specs=any_spec,
        out_shape=jax.ShapeDtypeStruct((sections, _G, _P, C), x.dtype),
        scratch_shapes=[
            pltpu.VMEM((sections, _G, _P, C), x.dtype),
            pltpu.VMEM((C, C), w.dtype),
            pltpu.VMEM((C,), b.dtype),
            pltpu.SemaphoreType.DMA((_AHEAD + 1,)),
            pltpu.SemaphoreType.DMA((_BULK,)),
            pltpu.SemaphoreType.DMA(()),
            pltpu.SemaphoreType.DMA(()),
            pltpu.SemaphoreType.DMA((2,)),
        ],
        compiler_params=pltpu.CompilerParams(
            vmem_limit_bytes=120 * 1024 * 1024,
            disable_bounds_checks=True,
        ),
    )(x.reshape(sections, _G, _P, C), w.reshape(C, C), b)
    return out.reshape(B, H, W, C)
```

```python
import jax
import jax.numpy as jnp
import jax.experimental.pallas as pl
import jax.experimental.pallas.tpu as pltpu
from jax import lax

_GROUPS = 6
_GROUP = 4096
_BLOCK = 128
_LANES = 128

_READ_PIECES = (40, 48, 40)
_FIRST_PIECES = (16,) * 8
_WRITE_PIECES = (32, 32, 32, 32)
_SMALL_SLOTS = (0, 0, 1, 2, 3, 4, 5, 7, 8, 10, 11, 12, 13, 14, 16, 17)
_FIRST_WRITE_SLOT = 13
_AHEAD = 2
_PRE_WRITE = 4


def _pieces(sizes):
    assert sum(sizes) == _BLOCK
    return [(sum(sizes[:i]), size) for i, size in enumerate(sizes)]


@jax.jit
def pallas_standalone__standard_2d_1d_3d_conv__vision_kernel(
    x: jax.Array,
    w: jax.Array,
    b: jax.Array,
):
    B, H, W, C = x.shape
    assert w.shape == (1, 1, C, C) and C % _LANES == 0
    sections = B * H * W // (2 * _GROUPS * _GROUP)
    assert sections * 2 * _GROUPS * _GROUP == B * H * W
    steps_per_section = _GROUP // _BLOCK
    steps = sections * steps_per_section
    bulk_groups = 2 * _GROUPS - 1
    small_rows = _BLOCK // len(_SMALL_SLOTS)
    lane_tiles = C // _LANES
    assert max(_SMALL_SLOTS + (_FIRST_WRITE_SLOT,)) <= _GROUPS * lane_tiles

    def kernel_function(x_hbm, w_hbm, b_hbm, o_hbm, buf, w_v, b_v,
                        bulk_sems, first_sems, small_sem, write_sem, param_sems):
        def locate(step, offset=0, size=_BLOCK):
            if isinstance(step, int):
                section, j = divmod(step, steps_per_section)
                return section, pl.ds(j * _BLOCK + offset, size)
            section = lax.shift_right_logical(step, steps_per_section.bit_length() - 1)
            j = step & (steps_per_section - 1)
            return section, pl.ds(pl.multiple_of(j * _BLOCK + offset, 8), size)

        def block_groups(block):
            upper = block >= steps
            if not isinstance(block, int):
                upper = upper.astype(jnp.int32)
            return block - upper * steps, pl.ds(upper * _GROUPS, _GROUPS)

        def bulk_read(step, sem, offset=0, size=_BLOCK):
            section, rows = locate(step, offset, size)
            ix = (section, pl.ds(0, bulk_groups), rows)
            return pltpu.make_async_copy(x_hbm.at[ix], buf.at[ix], sem)

        def start_bulk_reads(step, sem):
            for offset, size in _pieces(_READ_PIECES):
                bulk_read(step, sem, offset, size).start(priority=1)

        def start_small_read(step, q):
            section, rows = locate(step, q * small_rows, small_rows)
            ix = (section, bulk_groups, rows)
            pltpu.make_async_copy(x_hbm.at[ix], buf.at[ix], small_sem).start(priority=0)

        def start_writes(block):
            step, groups = block_groups(block)
            for offset, size in _pieces(_WRITE_PIECES):
                section, rows = locate(step, offset, size)
                ix = (section, groups, rows)
                pltpu.make_async_copy(buf.at[ix], o_hbm.at[ix], write_sem).start()

        def conv(xv):
            acc = jnp.dot(xv, w_v[...], preferred_element_type=jnp.float32)
            acc = acc + b_v[...].astype(jnp.float32).reshape(1, C)
            return acc.astype(buf.dtype)

        def compute(block):
            step, groups = block_groups(block)
            section, rows = locate(step)
            xv = buf[section, groups, rows, :].reshape(_GROUPS * _BLOCK, C)
            buf[section, groups, rows, :] = conv(xv).reshape(_GROUPS, _BLOCK, C)

        def compute_and_read(block):
            section, rows = locate(block)
            start_small_read(block + 1, 0)
            issued = 1
            xv = buf[section, 0, rows, :]
            for g in range(_GROUPS):
                ahead = buf[section, g + 1, rows, :] if g + 1 < _GROUPS else None
                if g == 0:
                    start_small_read(block + 1, 1)
                    issued = 2
                y = conv(xv)
                for t in range(lane_tiles):
                    lanes = slice(t * _LANES, (t + 1) * _LANES)
                    buf[section, g, rows, lanes] = y[:, lanes]
                    stored = g * lane_tiles + t + 1
                    while issued < len(_SMALL_SLOTS) and _SMALL_SLOTS[issued] <= stored:
                        start_small_read(block + 1, issued)
                        issued += 1
                    if stored == _FIRST_WRITE_SLOT:
                        pl.when(block == steps - 2)(lambda: start_writes(0))
                xv = ahead
            assert issued == len(_SMALL_SLOTS)

        copy_w = pltpu.make_async_copy(w_hbm, w_v, param_sems.at[0])
        copy_b = pltpu.make_async_copy(b_hbm, b_v, param_sems.at[1])
        first_reads = [
            bulk_read(0, first_sems.at[i], offset, size)
            for i, (offset, size) in enumerate(_pieces(_FIRST_PIECES))
        ]
        first_reads[0].start(priority=1)
        copy_w.start()
        copy_b.start()
        for read in first_reads[1:]:
            read.start(priority=1)
        for step in range(1, _AHEAD):
            start_bulk_reads(step, bulk_sems.at[step])
        per_wait = len(_SMALL_SLOTS) // len(first_reads)
        for i, read in enumerate(first_reads):
            for q in range(per_wait):
                start_small_read(0, i * per_wait + q)
            read.wait()
        copy_w.wait()
        copy_b.wait()

        def read_step(step, _):
            sem = bulk_sems.at[lax.rem(step, _AHEAD)]
            pl.when(step > 0)(lambda: bulk_read(step, sem).wait())
            pl.when(step + _AHEAD < steps)(lambda: start_bulk_reads(step + _AHEAD, sem))
            compute_and_read(step)

        lax.fori_loop(0, steps - 1, read_step, None)

        for block in range(1, _PRE_WRITE):
            start_writes(block)
        bulk_read(steps - 1, bulk_sems.at[(steps - 1) % _AHEAD]).wait()
        pltpu.make_async_copy(
            x_hbm.at[:, bulk_groups], buf.at[:, bulk_groups], small_sem).wait()

        computed = steps - 1
        assert _PRE_WRITE + 2 * (2 * steps - computed) >= 2 * steps

        def write_step(block, written):
            compute(block)
            target = jnp.minimum(block + 1, _PRE_WRITE + 2 * (block + 1 - computed))
            lax.fori_loop(written, target, lambda k, _: start_writes(k), None)
            return target

        lax.fori_loop(computed, 2 * steps, write_step, jnp.int32(_PRE_WRITE))
        pltpu.make_async_copy(buf, o_hbm, write_sem).wait()

    view = (sections, 2 * _GROUPS, _GROUP, C)
    any_spec = pl.BlockSpec(memory_space=pl.ANY)
    out = pl.pallas_call(
        kernel_function,
        in_specs=[any_spec, any_spec, any_spec],
        out_specs=any_spec,
        out_shape=jax.ShapeDtypeStruct(view, x.dtype),
        scratch_shapes=[
            pltpu.VMEM(view, x.dtype),
            pltpu.VMEM((C, C), w.dtype),
            pltpu.VMEM((C,), b.dtype),
            pltpu.SemaphoreType.DMA((_AHEAD,)),
            pltpu.SemaphoreType.DMA((len(_FIRST_PIECES),)),
            pltpu.SemaphoreType.DMA(()),
            pltpu.SemaphoreType.DMA(()),
            pltpu.SemaphoreType.DMA((2,)),
        ],
        compiler_params=pltpu.CompilerParams(vmem_limit_bytes=120 * 1024 * 1024),
    )(x.reshape(view), w.reshape(C, C), b)
    return out.reshape(B, H, W, C)
```

```python
import jax
import jax.numpy as jnp
import numpy as np
import jax.experimental.pallas as pl
import jax.experimental.pallas.tpu as pltpu
from jax import lax

_GROUPS = 6
_GROUP = 4096
_BLOCK = 128
_LANES = 128

_READ_PIECES = (40, 48, 40)
_FIRST_PIECES = (32, 32, 32, 32)
_WRITE_PIECES = (24, 40, 40, 24)
_SMALL_SLOTS = (0, 0, 1, 2, 3, 4, 5, 7, 8, 10, 11, 12, 13, 14, 16, 17)
_FIRST_WRITE_SLOT = 12
_AHEAD = 2
_PRE_WRITE = 4


def _pieces(sizes):
    assert sum(sizes) == _BLOCK
    return [(sum(sizes[:i]), size) for i, size in enumerate(sizes)]


@jax.jit
def pallas_standalone__standard_2d_1d_3d_conv__vision_kernel(
    x: jax.Array,
    w: jax.Array,
    b: jax.Array,
):
    B, H, W, C = x.shape
    assert w.shape == (1, 1, C, C) and C % _LANES == 0
    sections = B * H * W // (2 * _GROUPS * _GROUP)
    assert sections * 2 * _GROUPS * _GROUP == B * H * W
    steps_per_section = _GROUP // _BLOCK
    steps = sections * steps_per_section
    bulk_groups = 2 * _GROUPS - 1
    small_rows = _BLOCK // len(_SMALL_SLOTS)
    lane_tiles = C // _LANES
    assert max(_SMALL_SLOTS + (_FIRST_WRITE_SLOT,)) <= _GROUPS * lane_tiles

    def kernel_function(x_hbm, w_hbm, b_hbm, o_hbm, buf, w_v, b_v,
                        bulk_sems, first_sems, small_sem, write_sem, param_sems):
        def locate(step, offset=0, size=_BLOCK):
            if isinstance(step, int):
                section, j = divmod(step, steps_per_section)
                return section, pl.ds(j * _BLOCK + offset, size)
            section = lax.shift_right_logical(step, steps_per_section.bit_length() - 1)
            j = step & (steps_per_section - 1)
            return section, pl.ds(pl.multiple_of(j * _BLOCK + offset, 8), size)

        def block_groups(block):
            upper = block >= steps
            if not isinstance(block, int):
                upper = upper.astype(jnp.int32)
            return block - upper * steps, pl.ds(upper * _GROUPS, _GROUPS)

        def bulk_read(step, sem, offset=0, size=_BLOCK):
            section, rows = locate(step, offset, size)
            ix = (section, pl.ds(0, bulk_groups), rows)
            return pltpu.make_async_copy(x_hbm.at[ix], buf.at[ix], sem)

        def start_bulk_reads(step, sem):
            for offset, size in _pieces(_READ_PIECES):
                bulk_read(step, sem, offset, size).start(priority=1)

        def start_small_read(step, q):
            section, rows = locate(step, q * small_rows, small_rows)
            ix = (section, bulk_groups, rows)
            pltpu.make_async_copy(x_hbm.at[ix], buf.at[ix], small_sem).start(priority=0)

        def start_writes(block):
            step, groups = block_groups(block)
            for offset, size in _pieces(_WRITE_PIECES):
                section, rows = locate(step, offset, size)
                ix = (section, groups, rows)
                pltpu.make_async_copy(buf.at[ix], o_hbm.at[ix], write_sem).start()

        def conv(xv):
            acc = jnp.dot(xv, w_v[...], preferred_element_type=jnp.float32)
            acc = acc + b_v[...].astype(jnp.float32).reshape(1, C)
            return acc.astype(buf.dtype)

        def compute(block):
            step, groups = block_groups(block)
            section, rows = locate(step)
            xv = buf[section, groups, rows, :].reshape(_GROUPS * _BLOCK, C)
            buf[section, groups, rows, :] = conv(xv).reshape(_GROUPS, _BLOCK, C)

        def compute_and_read(block):
            section, rows = locate(block)
            start_small_read(block + 1, 0)
            issued = 1
            xv = buf[section, 0, rows, :]
            for g in range(_GROUPS):
                ahead = buf[section, g + 1, rows, :] if g + 1 < _GROUPS else None
                if g == 0:
                    start_small_read(block + 1, 1)
                    issued = 2
                y = conv(xv)
                for t in range(lane_tiles):
                    lanes = slice(t * _LANES, (t + 1) * _LANES)
                    buf[section, g, rows, lanes] = y[:, lanes]
                    stored = g * lane_tiles + t + 1
                    while issued < len(_SMALL_SLOTS) and _SMALL_SLOTS[issued] <= stored:
                        if stored < _FIRST_WRITE_SLOT:
                            start_small_read(block + 1, issued)
                        else:
                            pl.when(block < steps - 2)(
                                lambda q=issued: start_small_read(block + 1, q))
                        issued += 1
                    if stored == _FIRST_WRITE_SLOT:
                        pl.when(block == steps - 2)(lambda: start_writes(0))
                xv = ahead
            assert issued == len(_SMALL_SLOTS)

        copy_w = pltpu.make_async_copy(w_hbm, w_v, param_sems.at[0])
        copy_b = pltpu.make_async_copy(b_hbm, b_v, param_sems.at[1])
        first_reads = [
            bulk_read(0, first_sems.at[i], offset, size)
            for i, (offset, size) in enumerate(_pieces(_FIRST_PIECES))
        ]
        first_reads[0].start(priority=1)
        copy_w.start()
        copy_b.start()
        for read in first_reads[1:]:
            read.start(priority=1)
        for step in range(1, _AHEAD):
            start_bulk_reads(step, bulk_sems.at[step])
        per_wait = len(_SMALL_SLOTS) // len(first_reads)
        for i, read in enumerate(first_reads):
            for q in range(per_wait):
                start_small_read(0, i * per_wait + q)
            read.wait()
        for q, slot in enumerate(_SMALL_SLOTS):
            if slot >= _FIRST_WRITE_SLOT:
                start_small_read(steps - 1, q)
        copy_w.wait()
        copy_b.wait()

        def read_step(step, _):
            sem = bulk_sems.at[lax.rem(step, _AHEAD)]
            pl.when(step > 0)(lambda: bulk_read(step, sem).wait())
            pl.when(step + _AHEAD < steps)(lambda: start_bulk_reads(step + _AHEAD, sem))
            compute_and_read(step)

        lax.fori_loop(0, steps - 1, read_step, None)

        for block in range(1, _PRE_WRITE):
            start_writes(block)
        bulk_read(steps - 1, bulk_sems.at[(steps - 1) % _AHEAD]).wait()
        pltpu.make_async_copy(
            x_hbm.at[:, bulk_groups], buf.at[:, bulk_groups], small_sem).wait()

        computed = steps - 1
        assert _PRE_WRITE + 2 * (2 * steps - computed) >= 2 * steps

        def write_step(block, written):
            compute(block)
            target = jnp.minimum(block + 1, _PRE_WRITE + 2 * (block + 1 - computed))
            lax.fori_loop(written, target, lambda k, _: start_writes(k), None)
            return target

        lax.fori_loop(computed, 2 * steps, write_step, np.int32(_PRE_WRITE))
        pltpu.make_async_copy(buf, o_hbm, write_sem).wait()

    view = (sections, 2 * _GROUPS, _GROUP, C)
    any_spec = pl.BlockSpec(memory_space=pl.ANY)
    out = pl.pallas_call(
        kernel_function,
        in_specs=[any_spec, any_spec, any_spec],
        out_specs=any_spec,
        out_shape=jax.ShapeDtypeStruct(view, x.dtype),
        scratch_shapes=[
            pltpu.VMEM(view, x.dtype),
            pltpu.VMEM((C, C), w.dtype),
            pltpu.VMEM((C,), b.dtype),
            pltpu.SemaphoreType.DMA((_AHEAD,)),
            pltpu.SemaphoreType.DMA((len(_FIRST_PIECES),)),
            pltpu.SemaphoreType.DMA(()),
            pltpu.SemaphoreType.DMA(()),
            pltpu.SemaphoreType.DMA((2,)),
        ],
        compiler_params=pltpu.CompilerParams(vmem_limit_bytes=120 * 1024 * 1024),
    )(x.reshape(view), w.reshape(C, C), b)
    return out.reshape(B, H, W, C)
```
